```python
import os as _os
_os.environ.setdefault("JAX_PLATFORMS", "cpu")
import jax
import jax.numpy as jnp

def _softmax(x, axis=-1):
    return jax.nn.softmax(x, axis=axis)
def _gelu(x):
    return jax.nn.gelu(x, approximate=True)
def _silu(x):
    return jax.nn.silu(x)
def _sigmoid(x):
    return jax.nn.sigmoid(x)
def _layernorm(x, axis=-1, eps=1e-5):
    m = jnp.mean(x, axis=axis, keepdims=True)
    v = jnp.var(x, axis=axis, keepdims=True)
    return (x - m) / jnp.sqrt(v + eps)
def _scatter_add(tgt, idx, src, axis=0):
    return tgt.at[idx].add(src)
def _segment_sum(src, seg, n):
    return jax.ops.segment_sum(src, seg, n)
class _Rng:
    def __init__(self, key):
        self._k = key
    def _next(self):
        self._k, sub = jax.random.split(self._k)
        return sub
    def normal(self, shape):
        return jax.random.normal(self._next(), shape, dtype=jnp.bfloat16)
    def randint(self, lo, hi, shape):
        return jax.random.randint(self._next(), shape, lo, hi, dtype=jnp.int32)
    def uniform(self, shape, lo=0.0, hi=1.0):
        return jax.random.uniform(self._next(), shape, jnp.bfloat16, lo, hi)
    def permutation(self, n):
        return jax.random.permutation(self._next(), n)


kernel_name = 'sequential_preLN__linear_kernel_hedgehog__dense_activation_squared_relu__prompt'

def setup_inputs():
    _rng = _Rng(jax.random.key(int.from_bytes(__import__("os").urandom(4), "little")))
    _w = (lambda a: (lambda t: t.astype(jnp.bfloat16) if jnp.issubdtype(t.dtype, jnp.floating) else t)(jnp.asarray(a)))
    def _A_setup():
        B, S, D, H = 1, 2048, 512, 32
        Dh = D // H
        return {
            "x": _w((lambda *s: _rng.normal(s) * 0.05)(B, S, D)),
            "wqkv": _w((lambda *s: _rng.normal(s) * 0.2)(D, 3 * D)),
            "w_phi": _w((lambda *s: _rng.normal(s) * 0.2)(H, Dh, Dh) * (Dh ** -0.5)),
            "wo": _w((lambda *s: _rng.normal(s) * 0.05)(D, D)),
        }
    _A_in = _A_setup()

    def _B_setup():
        B, S, D, F = 1, 2048, 512, 1792
        return {
            "x": _w((lambda *s: _rng.normal(s) * 0.05)(B, S, D)),
            "w1": _w((lambda *s: _rng.normal(s) * 0.05)(D, F)),
            "b1": _w((lambda *s: _rng.normal(s) * 0.05)(F)),
            "w2": _w((lambda *s: _rng.normal(s) * 0.05)(F, D)),
            "b2": _w((lambda *s: _rng.normal(s) * 0.05)(D)),
        }
    _B_in = _B_setup()

    return {
        "A_x": _A_in["x"],
        "A_wqkv": _A_in["wqkv"],
        "A_w_phi": _A_in["w_phi"],
        "A_wo": _A_in["wo"],
        "B_x": _B_in["x"],
        "B_w1": _B_in["w1"],
        "B_b1": _B_in["b1"],
        "B_w2": _B_in["w2"],
        "B_b2": _B_in["b2"],
    }

def reference(A_x, A_wqkv, A_w_phi, A_wo, B_x, B_w1, B_b1, B_w2, B_b2):
    def _A_ref(x, wqkv, w_phi, wo):
        B, S, D = x.shape
        H = 32; Dh = D // H
        qkv = (lambda x, *d: x.transpose(*d))((x @ wqkv).reshape(B, S, 3, H, Dh), 2, 0, 3, 1, 4)
        q, k, v = qkv[0], qkv[1], qkv[2]
        pq = jnp.einsum("bhsd,hdf->bhsf", q, w_phi)
        pk = jnp.einsum("bhsd,hdf->bhsf", k, w_phi)
        phi_q = jnp.concatenate([_softmax(pq, axis=-1), _softmax(-pq, axis=-1)], axis=-1)
        phi_k = jnp.concatenate([_softmax(pk, axis=-1), _softmax(-pk, axis=-1)], axis=-1)
        kv = jnp.einsum("bhsf,bhsd->bhfd", phi_k, v)
        z  = jnp.einsum("bhsf->bhf", phi_k)
        num = jnp.einsum("bhqf,bhfd->bhqd", phi_q, kv)
        den = jnp.einsum("bhqf,bhf->bhq", phi_q, z)[..., None] + 1e-6
        o = num / den
        return (lambda x, *d: x.transpose(*d))(o, 0, 2, 1, 3).reshape(B, S, D) @ wo

    def _B_ref(x, w1, b1, w2, b2):
        h = jnp.einsum("bsd,df->bsf", x, w1) + b1
        zero = jnp.zeros_like(h)
        r = jnp.where(h > zero, h, zero)
        h = r * r
        out = jnp.einsum("bsf,fd->bsd", h, w2) + b2
        return out

    x = A_x
    h = x + _A_ref(_layernorm(x, axis=-1), A_wqkv, A_w_phi, A_wo)
    h2 = h + _B_ref(_layernorm(h, axis=-1), B_w1, B_b1, B_w2, B_b2)
    return h2
```

```python
import functools
import jax
import jax.numpy as jnp
from jax import lax
import jax.experimental.pallas as pl
import jax.experimental.pallas.tpu as pltpu

S, D, H, DH, F = 2048, 512, 32, 16, 1792
G = 4
TS = 512
NT = S // TS
EPS = 1e-5

_NT = (((1,), (1,)), ((), ()))
_NN = (((1,), (0,)), ((), ()))
_TN = (((0,), (0,)), ((), ()))


def _dot(a, b, dn):
    return lax.dot_general(a, b, dn, preferred_element_type=jnp.float32)


def _ln(x):
    m = jnp.mean(x, axis=-1, keepdims=True)
    xc = x - m
    v = jnp.mean(xc * xc, axis=-1, keepdims=True)
    return xc * lax.rsqrt(v + EPS)


def _kernel(x_hbm, wqkv_hbm, wphi_hbm, wo_hbm, w1_hbm, b1_hbm, w2_hbm, b2_hbm,
            out_hbm,
            x_v, wqkv_v, wphi_v, wo_v, w1_v, b1_v, w2_v, b2_v,
            wallT, woP, phiq, kv_acc, z_acc, lmat, out_v, sems, osems):
    cp_wphi = pltpu.make_async_copy(wphi_hbm, wphi_v, sems.at[0])
    cp_wqkv = pltpu.make_async_copy(wqkv_hbm, wqkv_v, sems.at[1])
    cp_x = pltpu.make_async_copy(x_hbm, x_v, sems.at[2])
    cp_wo = pltpu.make_async_copy(wo_hbm, wo_v, sems.at[3])
    cp_w1 = pltpu.make_async_copy(w1_hbm, w1_v, sems.at[4])
    cp_b1 = pltpu.make_async_copy(b1_hbm, b1_v, sems.at[5])
    cp_w2 = pltpu.make_async_copy(w2_hbm, w2_v, sems.at[6])
    cp_b2 = pltpu.make_async_copy(b2_hbm, b2_v, sems.at[7])
    cp_wphi.start()
    cp_wqkv.start()
    cp_x.start()
    cp_wphi.wait()
    cp_wqkv.wait()
    cp_wo.start()
    cp_w1.start()
    cp_b1.start()
    cp_w2.start()
    cp_b2.start()

    r = lax.broadcasted_iota(jnp.int32, (128, 128), 0)
    c = lax.broadcasted_iota(jnp.int32, (128, 128), 1)
    same_head = (r % 8) == (c // 16)
    perm = jnp.where(same_head & ((r // 8) == (c % 16)), 1.0, 0.0).astype(jnp.bfloat16)
    sr = lax.broadcasted_iota(jnp.int32, (32, 512), 0)
    sc = lax.broadcasted_iota(jnp.int32, (32, 512), 1)
    sel = jnp.where(sr == (sc // 16), 1.0, 0.0).astype(jnp.bfloat16)
    br = lax.broadcasted_iota(jnp.int32, (256, 512), 0)
    bc = lax.broadcasted_iota(jnp.int32, (256, 512), 1)
    bmat = jnp.where((br // 16) == (bc % 16), _dot(wphi_v[...], sel, _NN), 0.0).astype(jnp.bfloat16)
    er = lax.broadcasted_iota(jnp.int32, (128, 256), 0)
    ec = lax.broadcasted_iota(jnp.int32, (128, 256), 1)
    emat = jnp.where((er // 8) == (ec % 16), 1.0, 0.0).astype(jnp.bfloat16)
    tr = lax.broadcasted_iota(jnp.int32, (128, 512), 0)
    tc = lax.broadcasted_iota(jnp.int32, (128, 512), 1)
    tall = jnp.where((tr % 8) == ((tc // 16) % 8), _dot(emat, bmat, _NN), 0.0).astype(jnp.bfloat16)
    for g in range(G):
        tg = tall[:, g * 128:(g + 1) * 128]
        wallT[pl.ds(g * 128, 128), :] = _dot(tg, wqkv_v[:, pl.ds(g * 128, 128)], _NT).astype(jnp.bfloat16)
        wallT[pl.ds(512 + g * 128, 128), :] = _dot(tg, wqkv_v[:, pl.ds(512 + g * 128, 128)], _NT).astype(jnp.bfloat16)
        wallT[pl.ds(1024 + g * 128, 128), :] = _dot(perm, wqkv_v[:, pl.ds(1024 + g * 128, 128)], _NT).astype(jnp.bfloat16)

    kv_acc[...] = jnp.zeros_like(kv_acc)
    z_acc[...] = jnp.zeros_like(z_acc)
    cp_x.wait()

    def feat(p):
        p3 = p.reshape(16, 8, TS)
        mx = jnp.max(p3, axis=0, keepdims=True)
        mn = jnp.min(p3, axis=0, keepdims=True)
        ep = jnp.exp(p3 - mx)
        en = jnp.exp(mn - p3)
        sp = jnp.sum(ep, axis=0, keepdims=True)
        sn = jnp.sum(en, axis=0, keepdims=True)
        pp = (ep * (1.0 / sp)).reshape(128, TS)
        pn = (en * (1.0 / sn)).reshape(128, TS)
        return jnp.concatenate([pp, pn], axis=0)

    def phase1(t, carry):
        s0 = pl.multiple_of(t * TS, TS)
        xn = _ln(x_v[pl.ds(s0, TS), :].astype(jnp.float32)).astype(jnp.bfloat16)
        qkvT = _dot(wallT[...], xn, _NT)
        for g in range(G):
            pq = feat(qkvT[g * 128:(g + 1) * 128])
            phiq[t, pl.ds(g * 256, 256), :] = pq.astype(jnp.bfloat16)
            pk = feat(qkvT[512 + g * 128:512 + (g + 1) * 128])
            vT = qkvT[1024 + g * 128:1024 + (g + 1) * 128].astype(jnp.bfloat16)
            kv_acc[g] += _dot(pk.astype(jnp.bfloat16), vT, _NT)
            zp = pk[:, 0:128]
            for j in range(1, TS // 128):
                zp = zp + pk[:, j * 128:(j + 1) * 128]
            z_acc[g] += zp
        return carry

    lax.fori_loop(0, NT, phase1, 0)

    rr = lax.broadcasted_iota(jnp.int32, (128, 256), 0)
    cc = lax.broadcasted_iota(jnp.int32, (128, 256), 1)
    m_kv = (rr % 8) == (cc % 8)
    r8 = lax.broadcasted_iota(jnp.int32, (16, 256), 0)
    c8 = lax.broadcasted_iota(jnp.int32, (16, 256), 1)
    m_z = r8 == (c8 % 8)
    for g in range(G):
        kvT = kv_acc[g].T
        lmat[g, pl.ds(0, 128), :] = jnp.where(m_kv, kvT, 0.0).astype(jnp.bfloat16)
        zrow = jnp.sum(z_acc[g].T, axis=0, keepdims=True)
        lmat[g, pl.ds(128, 16), :] = jnp.where(m_z, jnp.broadcast_to(zrow, (16, 256)), 0.0).astype(jnp.bfloat16)

    cp_wo.wait()
    for g in range(G):
        woP[pl.ds(g * 128, 128), :] = _dot(perm, wo_v[pl.ds(g * 128, 128), :], _NN).astype(jnp.bfloat16)
    cp_w1.wait()
    cp_b1.wait()
    cp_w2.wait()
    cp_b2.wait()

    def out_copy(t):
        s0 = pl.multiple_of(t * TS, TS)
        return pltpu.make_async_copy(out_v.at[pl.ds(s0, TS), :], out_hbm.at[pl.ds(s0, TS), :], osems.at[t])

    def phase2(t, carry):
        s0 = pl.multiple_of(t * TS, TS)
        parts = []
        for g in range(G):
            nd = _dot(lmat[g], phiq[t, pl.ds(g * 256, 256), :], _NN)
            den = nd[128:136] + 1e-6
            o3 = nd[0:128].reshape(16, 8, TS) * (1.0 / den)[None]
            parts.append(o3.reshape(128, TS).astype(jnp.bfloat16))
        oT = jnp.concatenate(parts, axis=0)
        attn = _dot(oT, woP[...], _TN)
        h = x_v[pl.ds(s0, TS), :].astype(jnp.float32) + attn
        hn = _ln(h).astype(jnp.bfloat16)
        a = _dot(hn, w1_v[...], _NN) + b1_v[...].astype(jnp.float32).reshape(1, F)
        a = jnp.maximum(a, 0.0)
        a = (a * a).astype(jnp.bfloat16)
        y = _dot(a, w2_v[...], _NN) + b2_v[...].astype(jnp.float32).reshape(1, D) + h
        out_v[pl.ds(s0, TS), :] = y.astype(jnp.bfloat16)
        out_copy(t).start()
        return carry

    lax.fori_loop(0, NT, phase2, 0)
    for t in range(NT):
        out_copy(t).wait()


@jax.jit
def pallas_sequential_preLN__linear_kernel_hedgehog__dense_activation_squared_relu__prompt_kernel(
    A_x, A_wqkv, A_w_phi, A_wo, B_x, B_w1, B_b1, B_w2, B_b2,
):
    bf = jnp.bfloat16
    x2 = A_x.reshape(S, D)
    wphi2 = jnp.transpose(A_w_phi, (1, 2, 0)).reshape(DH * DH, H)
    b1 = B_b1
    b2 = B_b2
    any_spec = pl.BlockSpec(memory_space=pl.ANY)
    out = pl.pallas_call(
        _kernel,
        out_shape=jax.ShapeDtypeStruct((S, D), bf),
        in_specs=[any_spec] * 8,
        out_specs=any_spec,
        scratch_shapes=[
            pltpu.VMEM((S, D), bf),
            pltpu.VMEM((D, 3 * D), bf),
            pltpu.VMEM((DH * DH, H), bf),
            pltpu.VMEM((D, D), bf),
            pltpu.VMEM((D, F), bf),
            pltpu.VMEM((F,), bf),
            pltpu.VMEM((F, D), bf),
            pltpu.VMEM((D,), bf),
            pltpu.VMEM((3 * D, D), bf),
            pltpu.VMEM((D, D), bf),
            pltpu.VMEM((NT, 2 * D, TS), bf),
            pltpu.VMEM((G, 256, 128), jnp.float32),
            pltpu.VMEM((G, 256, 128), jnp.float32),
            pltpu.VMEM((G, 144, 256), bf),
            pltpu.VMEM((S, D), bf),
            pltpu.SemaphoreType.DMA((8,)),
            pltpu.SemaphoreType.DMA((NT,)),
        ],
        compiler_params=pltpu.CompilerParams(vmem_limit_bytes=100 * 1024 * 1024),
    )(x2, A_wqkv, wphi2, A_wo, B_w1, b1, B_w2, b2)
    return out.reshape(1, S, D)
```

```python
import functools
import jax
import jax.numpy as jnp
from jax import lax
import jax.experimental.pallas as pl
import jax.experimental.pallas.tpu as pltpu

S, D, H, DH, F = 2048, 512, 32, 16, 1792
G = 4
TS = 512
NT = S // TS
NH = 4
TH = 256
NT2 = S // (NH * TH)
EPS = 1e-5
LOG2E = 1.4426950408889634

_NT = (((1,), (1,)), ((), ()))
_NN = (((1,), (0,)), ((), ()))
_TN = (((0,), (0,)), ((), ()))


def _dot(a, b, dn):
    return lax.dot_general(a, b, dn, preferred_element_type=jnp.float32)


def _ln(x):
    m = jnp.mean(x, axis=-1, keepdims=True)
    xc = x - m
    v = jnp.mean(xc * xc, axis=-1, keepdims=True)
    return xc * lax.rsqrt(v + EPS)


def _feat(p, r):
    n = p.shape[-1]
    p3 = p.reshape(16, 8, n) * r[None]
    mx = jnp.max(p3, axis=0, keepdims=True)
    mn = jnp.min(p3, axis=0, keepdims=True)
    ep = jnp.exp2(p3 - mx)
    en = jnp.exp2(mn - p3)
    sp = jnp.sum(ep, axis=0, keepdims=True)
    sn = jnp.sum(en, axis=0, keepdims=True)
    pp = (ep * (1.0 / sp)).reshape(128, n)
    pn = (en * (1.0 / sn)).reshape(128, n)
    return jnp.concatenate([pp, pn], axis=0)


def _kernel(x_hbm, wqkv_hbm, wphi_hbm, wo_hbm, w1_hbm, b1_hbm, w2_hbm, b2_hbm,
            out_hbm,
            x_v, wq_v, wk_v, wv_v, wphi_v, wo_v, w1_v, b1_v, w2_v, b2_v,
            wqT, wkT, r_v, lmat, out_v, sems, xsems, osems):
    cp_wphi = pltpu.make_async_copy(wphi_hbm, wphi_v, sems.at[0])
    cp_wq = pltpu.make_async_copy(wqkv_hbm.at[:, pl.ds(0, D)], wq_v, sems.at[1])
    cp_wk = pltpu.make_async_copy(wqkv_hbm.at[:, pl.ds(D, D)], wk_v, sems.at[2])
    cp_wv = pltpu.make_async_copy(wqkv_hbm.at[:, pl.ds(2 * D, D)], wv_v, sems.at[8])
    cp_wo = pltpu.make_async_copy(wo_hbm, wo_v, sems.at[3])
    cp_w1 = pltpu.make_async_copy(w1_hbm, w1_v, sems.at[4])
    cp_b1 = pltpu.make_async_copy(b1_hbm, b1_v, sems.at[5])
    cp_w2 = pltpu.make_async_copy(w2_hbm, w2_v, sems.at[6])
    cp_b2 = pltpu.make_async_copy(b2_hbm, b2_v, sems.at[7])

    def x_copy(t):
        s0 = t * TS if isinstance(t, int) else pl.multiple_of(t * TS, TS)
        return pltpu.make_async_copy(x_hbm.at[pl.ds(s0, TS), :], x_v.at[pl.ds(s0, TS), :], xsems.at[t])

    cp_wphi.start()
    cp_wk.start()
    x_copy(0).start()
    cp_wv.start()
    x_copy(1).start()

    cp_wphi.wait()
    sr = lax.broadcasted_iota(jnp.int32, (32, 512), 0)
    sc = lax.broadcasted_iota(jnp.int32, (32, 512), 1)
    sel = jnp.where(sr == (sc // 16), 1.0, 0.0).astype(jnp.bfloat16)
    br = lax.broadcasted_iota(jnp.int32, (256, 512), 0)
    bc = lax.broadcasted_iota(jnp.int32, (256, 512), 1)
    bmat = jnp.where((br // 16) == (bc % 16), _dot(wphi_v[...], sel, _NN), 0.0).astype(jnp.bfloat16)
    er = lax.broadcasted_iota(jnp.int32, (128, 256), 0)
    ec = lax.broadcasted_iota(jnp.int32, (128, 256), 1)
    emat = jnp.where((er // 8) == (ec % 16), 1.0, 0.0).astype(jnp.bfloat16)
    tr = lax.broadcasted_iota(jnp.int32, (128, 512), 0)
    tc = lax.broadcasted_iota(jnp.int32, (128, 512), 1)
    tall = jnp.where((tr % 8) == ((tc // 16) % 8), _dot(emat, bmat, _NN), 0.0).astype(jnp.bfloat16)

    def fold(w_v, wT):
        for g in range(G):
            tg = tall[:, g * 128:(g + 1) * 128]
            w = _dot(tg, w_v[:, pl.ds(g * 128, 128)], _NT)
            w = w - jnp.mean(w, axis=-1, keepdims=True)
            wT[pl.ds(g * 128, 128), :] = w.astype(jnp.bfloat16)

    cp_wk.wait()
    fold(wk_v, wkT)

    def k_raw(t):
        xb = x_v[pl.ds(t * TS, TS), :]
        kT = _dot(wkT[...], xb, _NT)
        xf = xb.astype(jnp.float32)
        mu = jnp.mean(xf, axis=-1, keepdims=True)
        xc = xf - mu
        var = jnp.mean(xc * xc, axis=-1, keepdims=True)
        rc = lax.rsqrt(var + EPS)
        rr = jnp.broadcast_to(rc * LOG2E, (TS, 128)).T[0:8]
        r_v[t] = rr
        return kT, mu, rc, rr

    def rest(t, kT, mu, rc, rr, wvs, kvs, zs):
        vr = _dot(x_v[pl.ds(t * TS, TS), :], wv_v[...], _NN)
        v = ((vr - mu * wvs) * rc).astype(jnp.bfloat16)
        kvs_new, zs_new = [], []
        for g in range(G):
            pk = _feat(kT[g * 128:(g + 1) * 128], rr)
            zp = pk[:, 0:128]
            for j in range(1, TS // 128):
                zp = zp + pk[:, j * 128:(j + 1) * 128]
            kv = _dot(pk.astype(jnp.bfloat16), v[:, g * 128:(g + 1) * 128], _NN)
            kvs_new.append(kv if kvs is None else kvs[g] + kv)
            zs_new.append(zp if zs is None else zs[g] + zp)
        return kvs_new, zs_new

    x_copy(0).wait()
    x_copy(2).start()
    x_copy(3).start()
    cp_wq.start()
    k0 = k_raw(0)
    cp_wv.wait()
    x_copy(1).wait()
    cp_wo.start()
    cp_w1.start()
    cp_b1.start()
    cp_w2.start()
    cp_b2.start()
    wvs = _dot(jnp.ones((8, D), jnp.bfloat16), wv_v[...], _NN)[0:1]
    kvs, zs = rest(0, *k0, wvs, None, None)
    kvs, zs = rest(1, *k_raw(1), wvs, kvs, zs)
    x_copy(2).wait()
    x_copy(3).wait()
    cp_wq.wait()
    kvs, zs = rest(2, *k_raw(2), wvs, kvs, zs)
    kvs, zs = rest(3, *k_raw(3), wvs, kvs, zs)
    fold(wq_v, wqT)

    rr = lax.broadcasted_iota(jnp.int32, (128, 256), 0)
    cc = lax.broadcasted_iota(jnp.int32, (128, 256), 1)
    m_kv = (rr // 16) == (cc % 8)
    r8 = lax.broadcasted_iota(jnp.int32, (16, 256), 0)
    c8 = lax.broadcasted_iota(jnp.int32, (16, 256), 1)
    m_z = r8 == (c8 % 8)
    for g in range(G):
        kvT = kvs[g].T
        lmat[g, pl.ds(0, 128), :] = jnp.where(m_kv, kvT, 0.0).astype(jnp.bfloat16)
        zrow = jnp.sum(zs[g].T, axis=0, keepdims=True)
        lmat[g, pl.ds(128, 16), :] = jnp.where(m_z, jnp.broadcast_to(zrow, (16, 256)), 0.0).astype(jnp.bfloat16)

    cp_wo.wait()
    cp_w1.wait()
    cp_b1.wait()
    cp_w2.wait()
    cp_b2.wait()

    def out_copy(i):
        s0 = i * TH if isinstance(i, int) else pl.multiple_of(i * TH, TH)
        return pltpu.make_async_copy(out_v.at[pl.ds(s0, TH), :], out_hbm.at[pl.ds(s0, TH), :], osems.at[i])

    def phase2(t, carry):
        offs = [pl.multiple_of((t * NH + u) * TH, TH) for u in range(NH)]
        qTs = [_dot(wqT[...], x_v[pl.ds(s0, TH), :], _NT) for s0 in offs]
        oTs = []
        for u in range(NH):
            rr = r_v[t * (NH * TH // TS) + (u * TH) // TS, :, pl.ds((u * TH) % TS, TH)]
            parts = []
            for g in range(G):
                pq = _feat(qTs[u][g * 128:(g + 1) * 128], rr).astype(jnp.bfloat16)
                nd = _dot(lmat[g], pq, _NN)
                rden = 1.0 / (nd[128:136] + 1e-6)
                o3 = nd[0:128].reshape(8, 16, TH) * rden.reshape(8, 1, TH)
                parts.append(o3.reshape(128, TH).astype(jnp.bfloat16))
            oTs.append(jnp.concatenate(parts, axis=0))
        hs = []
        for u in range(NH):
            attn = _dot(oTs[u], wo_v[...], _TN)
            h = x_v[pl.ds(offs[u], TH), :].astype(jnp.float32) + attn
            hs.append((h, _ln(h).astype(jnp.bfloat16)))
        for u in range(NH):
            h, hn = hs[u]
            a = _dot(hn, w1_v[...], _NN) + b1_v[...].astype(jnp.float32).reshape(1, F)
            a = jnp.maximum(a, 0.0)
            a = (a * a).astype(jnp.bfloat16)
            y = _dot(a, w2_v[...], _NN) + b2_v[...].astype(jnp.float32).reshape(1, D) + h
            out_v[pl.ds(offs[u], TH), :] = y.astype(jnp.bfloat16)
            out_copy(t * NH + u).start()
        return carry

    lax.fori_loop(0, NT2, phase2, 0)
    for i in range(NT2 * NH):
        out_copy(i).wait()


@jax.jit
def pallas_sequential_preLN__linear_kernel_hedgehog__dense_activation_squared_relu__prompt_kernel(
    A_x, A_wqkv, A_w_phi, A_wo, B_x, B_w1, B_b1, B_w2, B_b2,
):
    bf = jnp.bfloat16
    x2 = A_x.reshape(S, D)
    wphi2 = jnp.transpose(A_w_phi, (1, 2, 0)).reshape(DH * DH, H)
    any_spec = pl.BlockSpec(memory_space=pl.ANY)
    out = pl.pallas_call(
        _kernel,
        out_shape=jax.ShapeDtypeStruct((S, D), bf),
        in_specs=[any_spec] * 8,
        out_specs=any_spec,
        scratch_shapes=[
            pltpu.VMEM((S, D), bf),
            pltpu.VMEM((D, D), bf),
            pltpu.VMEM((D, D), bf),
            pltpu.VMEM((D, D), bf),
            pltpu.VMEM((DH * DH, H), bf),
            pltpu.VMEM((D, D), bf),
            pltpu.VMEM((D, F), bf),
            pltpu.VMEM((F,), bf),
            pltpu.VMEM((F, D), bf),
            pltpu.VMEM((D,), bf),
            pltpu.VMEM((D, D), bf),
            pltpu.VMEM((D, D), bf),
            pltpu.VMEM((NT, 8, TS), jnp.float32),
            pltpu.VMEM((G, 144, 256), bf),
            pltpu.VMEM((S, D), bf),
            pltpu.SemaphoreType.DMA((9,)),
            pltpu.SemaphoreType.DMA((NT,)),
            pltpu.SemaphoreType.DMA((NT2 * NH,)),
        ],
        compiler_params=pltpu.CompilerParams(vmem_limit_bytes=100 * 1024 * 1024),
    )(x2, A_wqkv, wphi2, A_wo, B_w1, B_b1, B_w2, B_b2)
    return out.reshape(1, S, D)
```

```python
import functools
import jax
import jax.numpy as jnp
from jax import lax
import jax.experimental.pallas as pl
import jax.experimental.pallas.tpu as pltpu

S, D, H, DH, F = 2048, 512, 32, 16, 1792
G = 4
TS = 512
NT = S // TS
NH = 4
TH = 256
NT2 = S // (NH * TH)
EPS = 1e-5
LOG2E = 1.4426950408889634

_NT = (((1,), (1,)), ((), ()))
_NN = (((1,), (0,)), ((), ()))
_TN = (((0,), (0,)), ((), ()))


def _dot(a, b, dn):
    return lax.dot_general(a, b, dn, preferred_element_type=jnp.float32)


def _ln(x):
    m = jnp.mean(x, axis=-1, keepdims=True)
    xc = x - m
    v = jnp.mean(xc * xc, axis=-1, keepdims=True)
    return xc * lax.rsqrt(v + EPS)


def _feat(p, r, zb=None):
    n = p.shape[-1]
    p3 = p.reshape(16, 8, n) * r[None]
    mx = jnp.max(p3, axis=0, keepdims=True)
    mn = jnp.min(p3, axis=0, keepdims=True)
    ep = jnp.exp2(p3 - mx)
    en = jnp.exp2(mn - p3)
    sp = jnp.sum(ep, axis=0, keepdims=True)
    sn = jnp.sum(en, axis=0, keepdims=True)
    pp = ep * (1.0 / sp)
    pn = en * (1.0 / sn)
    phi = jnp.concatenate([pp.reshape(128, n), pn.reshape(128, n)], axis=0)
    if zb is None:
        return phi
    zt = jnp.concatenate([zb] * (n // 128), axis=1).reshape(2, 16, 8, n)
    den = jnp.sum(pp * zt[0], axis=0) + jnp.sum(pn * zt[1], axis=0)
    return phi, den


def _kernel(x_hbm, wqkv_hbm, wphi_hbm, wo_hbm, w1_hbm, b1_hbm, w2_hbm, b2_hbm,
            out_hbm,
            x_v, wq_v, wk_v, wv_v, wphi_v, wo_v, w1_v, b1_v, w2_v, b2_v,
            wqT, wkT, r_v, kv_s, z_s, out_v, sems, xsems, osems):
    cp_wphi = pltpu.make_async_copy(wphi_hbm, wphi_v, sems.at[0])
    cp_wq = pltpu.make_async_copy(wqkv_hbm.at[:, pl.ds(0, D)], wq_v, sems.at[1])
    cp_wk = pltpu.make_async_copy(wqkv_hbm.at[:, pl.ds(D, D)], wk_v, sems.at[2])
    cp_wv = pltpu.make_async_copy(wqkv_hbm.at[:, pl.ds(2 * D, D)], wv_v, sems.at[8])
    cp_wo = pltpu.make_async_copy(wo_hbm, wo_v, sems.at[3])
    cp_w1 = pltpu.make_async_copy(w1_hbm, w1_v, sems.at[4])
    cp_b1 = pltpu.make_async_copy(b1_hbm, b1_v, sems.at[5])
    cp_w2 = pltpu.make_async_copy(w2_hbm, w2_v, sems.at[6])
    cp_b2 = pltpu.make_async_copy(b2_hbm, b2_v, sems.at[7])

    def x_copy(t):
        s0 = t * TS if isinstance(t, int) else pl.multiple_of(t * TS, TS)
        return pltpu.make_async_copy(x_hbm.at[pl.ds(s0, TS), :], x_v.at[pl.ds(s0, TS), :], xsems.at[t])

    cp_wphi.start()
    cp_wk.start()
    x_copy(0).start()
    cp_wv.start()
    x_copy(1).start()

    cp_wphi.wait()
    sr = lax.broadcasted_iota(jnp.int32, (32, 512), 0)
    sc = lax.broadcasted_iota(jnp.int32, (32, 512), 1)
    sel = jnp.where(sr == (sc // 16), 1.0, 0.0).astype(jnp.bfloat16)
    br = lax.broadcasted_iota(jnp.int32, (256, 512), 0)
    bc = lax.broadcasted_iota(jnp.int32, (256, 512), 1)
    bmat = jnp.where((br // 16) == (bc % 16), _dot(wphi_v[...], sel, _NN), 0.0).astype(jnp.bfloat16)
    er = lax.broadcasted_iota(jnp.int32, (128, 256), 0)
    ec = lax.broadcasted_iota(jnp.int32, (128, 256), 1)
    emat = jnp.where((er // 8) == (ec % 16), 1.0, 0.0).astype(jnp.bfloat16)
    tr = lax.broadcasted_iota(jnp.int32, (128, 512), 0)
    tc = lax.broadcasted_iota(jnp.int32, (128, 512), 1)
    tall = jnp.where((tr % 8) == ((tc // 16) % 8), _dot(emat, bmat, _NN), 0.0).astype(jnp.bfloat16)

    def fold(w_v, wT):
        for g in range(G):
            tg = tall[:, g * 128:(g + 1) * 128]
            w = _dot(tg, w_v[:, pl.ds(g * 128, 128)], _NT)
            w = w - jnp.mean(w, axis=-1, keepdims=True)
            wT[pl.ds(g * 128, 128), :] = w.astype(jnp.bfloat16)

    cp_wk.wait()
    fold(wk_v, wkT)

    def k_raw(t):
        xb = x_v[pl.ds(t * TS, TS), :]
        kT = _dot(wkT[...], xb, _NT)
        xf = xb.astype(jnp.float32)
        mu = jnp.mean(xf, axis=-1, keepdims=True)
        xc = xf - mu
        var = jnp.mean(xc * xc, axis=-1, keepdims=True)
        rc = lax.rsqrt(var + EPS)
        rr = jnp.broadcast_to(rc * LOG2E, (TS, 128)).T[0:8]
        r_v[t] = rr
        return kT, mu, rc, rr

    def rest(t, kT, mu, rc, rr, wvs, kvs, zs):
        vr = _dot(x_v[pl.ds(t * TS, TS), :], wv_v[...], _NN)
        v = ((vr - mu * wvs) * rc).astype(jnp.bfloat16)
        kvs_new, zs_new = [], []
        for g in range(G):
            pk = _feat(kT[g * 128:(g + 1) * 128], rr)
            zp = pk[:, 0:128]
            for j in range(1, TS // 128):
                zp = zp + pk[:, j * 128:(j + 1) * 128]
            kv = _dot(pk.astype(jnp.bfloat16), v[:, g * 128:(g + 1) * 128], _NN)
            kvs_new.append(kv if kvs is None else kvs[g] + kv)
            zs_new.append(zp if zs is None else zs[g] + zp)
        return kvs_new, zs_new

    def half(t, hh, wvs, kvs, zs):
        T2 = TS // 2
        xb = x_v[pl.ds(t * TS + hh * T2, T2), :]
        kT = _dot(wkT[...], xb, _NT)
        vr = _dot(xb, wv_v[...], _NN)
        xf = xb.astype(jnp.float32)
        mu = jnp.mean(xf, axis=-1, keepdims=True)
        xc = xf - mu
        var = jnp.mean(xc * xc, axis=-1, keepdims=True)
        rc = lax.rsqrt(var + EPS)
        rr = jnp.broadcast_to(rc * LOG2E, (T2, 128)).T[0:8]
        r_v[t, :, pl.ds(hh * T2, T2)] = rr
        v = ((vr - mu * wvs) * rc).astype(jnp.bfloat16)
        kvs_new, zs_new = [], []
        for g in range(G):
            pk = _feat(kT[g * 128:(g + 1) * 128], rr)
            zp = pk[:, 0:128]
            for j in range(1, T2 // 128):
                zp = zp + pk[:, j * 128:(j + 1) * 128]
            kv = _dot(pk.astype(jnp.bfloat16), v[:, g * 128:(g + 1) * 128], _NN)
            kvs_new.append(kvs[g] + kv)
            zs_new.append(zs[g] + zp)
        return kvs_new, zs_new

    x_copy(0).wait()
    x_copy(2).start()
    x_copy(3).start()
    cp_wq.start()
    k0 = k_raw(0)
    cp_wv.wait()
    x_copy(1).wait()
    cp_wo.start()
    cp_w1.start()
    cp_b1.start()
    cp_w2.start()
    cp_b2.start()
    wvs = _dot(jnp.ones((8, D), jnp.bfloat16), wv_v[...], _NN)[0:1]
    kvs, zs = rest(0, *k0, wvs, None, None)
    kvs, zs = half(1, 0, wvs, kvs, zs)
    kvs, zs = half(1, 1, wvs, kvs, zs)
    x_copy(2).wait()
    x_copy(3).wait()
    cp_wq.wait()
    kvs, zs = half(2, 0, wvs, kvs, zs)
    kvs, zs = half(2, 1, wvs, kvs, zs)
    kvs, zs = half(3, 0, wvs, kvs, zs)
    fold(wq_v, wqT)
    kvs, zs = half(3, 1, wvs, kvs, zs)
    for g in range(G):
        kv_s[g] = kvs[g]
        z_s[g] = zs[g]

    cp_wo.wait()
    cp_w1.wait()
    cp_b1.wait()
    cp_w2.wait()
    cp_b2.wait()

    def out_copy(i, c=None):
        s0 = i * TH if isinstance(i, int) else pl.multiple_of(i * TH, TH)
        if c is None:
            return pltpu.make_async_copy(out_v.at[pl.ds(s0, TH), :], out_hbm.at[pl.ds(s0, TH), :], osems.at[i])
        cs = pl.ds(c * (D // 2), D // 2)
        sem = osems.at[i] if c == 0 else osems.at[NT2 * NH + i // NH]
        return pltpu.make_async_copy(out_v.at[pl.ds(s0, TH), cs], out_hbm.at[pl.ds(s0, TH), cs], sem)

    def phase2(t, carry):
        rr_ = lax.broadcasted_iota(jnp.int32, (128, 256), 0)
        cc_ = lax.broadcasted_iota(jnp.int32, (128, 256), 1)
        m_kv = (rr_ // 16) == (cc_ % 8)
        lmats = [jnp.where(m_kv, kv_s[g].T, 0.0).astype(jnp.bfloat16) for g in range(G)]
        zbs = [jnp.broadcast_to(jnp.sum(z_s[g], axis=1, keepdims=True), (256, 128)) for g in range(G)]
        offs = [pl.multiple_of((t * NH + u) * TH, TH) for u in range(NH)]
        qTs = [_dot(wqT[...], x_v[pl.ds(s0, TH), :], _NT) for s0 in offs]
        oTs = []
        for u in range(NH):
            rr = r_v[t * (NH * TH // TS) + (u * TH) // TS, :, pl.ds((u * TH) % TS, TH)]
            parts = []
            for g in range(G):
                pq, den = _feat(qTs[u][g * 128:(g + 1) * 128], rr, zbs[g])
                nd = _dot(lmats[g], pq.astype(jnp.bfloat16), _NN)
                rden = 1.0 / (den + 1e-6)
                o3 = nd.reshape(8, 16, TH) * rden.reshape(8, 1, TH)
                parts.append(o3.reshape(128, TH).astype(jnp.bfloat16))
            oTs.append(jnp.concatenate(parts, axis=0))
        hs = []
        for u in range(NH):
            attn = _dot(oTs[u], wo_v[...], _TN)
            h = x_v[pl.ds(offs[u], TH), :].astype(jnp.float32) + attn
            hs.append((h, _ln(h).astype(jnp.bfloat16)))
        for u in range(NH):
            h, hn = hs[u]
            a = _dot(hn, w1_v[...], _NN) + b1_v[...].astype(jnp.float32).reshape(1, F)
            a = jnp.maximum(a, 0.0)
            a = (a * a).astype(jnp.bfloat16)
            if u < NH - 1:
                y = _dot(a, w2_v[...], _NN) + b2_v[...].astype(jnp.float32).reshape(1, D) + h
                out_v[pl.ds(offs[u], TH), :] = y.astype(jnp.bfloat16)
                out_copy(t * NH + u).start()
            else:
                b2f = b2_v[...].astype(jnp.float32).reshape(1, D)
                for c in range(2):
                    lo, hi = c * (D // 2), (c + 1) * (D // 2)
                    y = _dot(a, w2_v[:, pl.ds(lo, D // 2)], _NN) + b2f[:, lo:hi] + h[:, lo:hi]
                    out_v[pl.ds(offs[u], TH), pl.ds(lo, D // 2)] = y.astype(jnp.bfloat16)
                    out_copy(t * NH + u, c).start()
        return carry

    lax.fori_loop(0, NT2, phase2, 0)
    for i in range(NT2 * NH):
        if i % NH < NH - 1:
            out_copy(i).wait()
        else:
            out_copy(i, 0).wait()
            out_copy(i, 1).wait()


@jax.jit
def pallas_sequential_preLN__linear_kernel_hedgehog__dense_activation_squared_relu__prompt_kernel(
    A_x, A_wqkv, A_w_phi, A_wo, B_x, B_w1, B_b1, B_w2, B_b2,
):
    bf = jnp.bfloat16
    x2 = A_x.reshape(S, D)
    wphi2 = jnp.transpose(A_w_phi, (1, 2, 0)).reshape(DH * DH, H)
    any_spec = pl.BlockSpec(memory_space=pl.ANY)
    out = pl.pallas_call(
        _kernel,
        out_shape=jax.ShapeDtypeStruct((S, D), bf),
        in_specs=[any_spec] * 8,
        out_specs=any_spec,
        scratch_shapes=[
            pltpu.VMEM((S, D), bf),
            pltpu.VMEM((D, D), bf),
            pltpu.VMEM((D, D), bf),
            pltpu.VMEM((D, D), bf),
            pltpu.VMEM((DH * DH, H), bf),
            pltpu.VMEM((D, D), bf),
            pltpu.VMEM((D, F), bf),
            pltpu.VMEM((F,), bf),
            pltpu.VMEM((F, D), bf),
            pltpu.VMEM((D,), bf),
            pltpu.VMEM((D, D), bf),
            pltpu.VMEM((D, D), bf),
            pltpu.VMEM((NT, 8, TS), jnp.float32),
            pltpu.VMEM((G, 256, 128), jnp.float32),
            pltpu.VMEM((G, 256, 128), jnp.float32),
            pltpu.VMEM((S, D), bf),
            pltpu.SemaphoreType.DMA((9,)),
            pltpu.SemaphoreType.DMA((NT,)),
            pltpu.SemaphoreType.DMA((NT2 * NH + NT2,)),
        ],
        compiler_params=pltpu.CompilerParams(vmem_limit_bytes=100 * 1024 * 1024),
    )(x2, A_wqkv, wphi2, A_wo, B_w1, B_b1, B_w2, B_b2)
    return out.reshape(1, S, D)
```

```python
import jax
import jax.numpy as jnp
from jax import lax
import jax.experimental.pallas as pl
import jax.experimental.pallas.tpu as pltpu

S, D, H, DH, F = 2048, 512, 32, 16, 1792
G = 4
TS = 512
NT = S // TS
NH = 4
TH = 256
NT2 = S // (NH * TH)
EPS = 1e-5
LOG2E = 1.4426950408889634

_NT = (((1,), (1,)), ((), ()))
_NN = (((1,), (0,)), ((), ()))
_TN = (((0,), (0,)), ((), ()))


def _dot(a, b, dn):
    return lax.dot_general(a, b, dn, preferred_element_type=jnp.float32)


def _ln(x):
    m = jnp.mean(x, axis=-1, keepdims=True)
    xc = x - m
    v = jnp.mean(xc * xc, axis=-1, keepdims=True)
    return xc * lax.rsqrt(v + EPS)


def _feat(p, r, zb=None):
    n = p.shape[-1]
    p3 = p.reshape(16, 8, n) * r[None]
    mx = jnp.max(p3, axis=0, keepdims=True)
    mn = jnp.min(p3, axis=0, keepdims=True)
    ep = jnp.exp2(p3 - mx)
    en = jnp.exp2(mn - p3)
    sp = jnp.sum(ep, axis=0, keepdims=True)
    sn = jnp.sum(en, axis=0, keepdims=True)
    pp = ep * (1.0 / sp)
    pn = en * (1.0 / sn)
    phi = jnp.concatenate([pp.reshape(128, n), pn.reshape(128, n)], axis=0)
    if zb is None:
        return phi
    zt = jnp.concatenate([zb] * (n // 128), axis=1).reshape(2, 16, 8, n)
    den = jnp.sum(pp * zt[0], axis=0) + jnp.sum(pn * zt[1], axis=0)
    return phi, den


def _kernel(x_hbm, wqkv_hbm, wphi_hbm, wo_hbm, w1_hbm, b1_hbm, w2_hbm, b2_hbm,
            out_hbm,
            x_v, wq_v, wk_v, wv_v, wphi_v, wo_v, w1_v, b1_v, w2_v, b2_v,
            wqT, wkT, r_v, kv_s, z_s, out_v, sems, xsems, osems):
    cp_wphi = pltpu.make_async_copy(wphi_hbm, wphi_v, sems.at[0])
    cp_wq = pltpu.make_async_copy(wqkv_hbm.at[:, pl.ds(0, D)], wq_v, sems.at[1])
    cp_wk = pltpu.make_async_copy(wqkv_hbm.at[:, pl.ds(D, D)], wk_v, sems.at[2])
    cp_wv = pltpu.make_async_copy(wqkv_hbm.at[:, pl.ds(2 * D, D)], wv_v, sems.at[8])
    cp_wo = pltpu.make_async_copy(wo_hbm, wo_v, sems.at[3])
    cp_w1 = pltpu.make_async_copy(w1_hbm, w1_v, sems.at[4])
    cp_b1 = pltpu.make_async_copy(b1_hbm, b1_v, sems.at[5])
    cp_w2 = pltpu.make_async_copy(w2_hbm, w2_v, sems.at[6])
    cp_b2 = pltpu.make_async_copy(b2_hbm, b2_v, sems.at[7])

    def x_copy(t):
        return pltpu.make_async_copy(x_hbm.at[pl.ds(t * TS, TS), :], x_v.at[pl.ds(t * TS, TS), :], xsems.at[t])

    cp_wphi.start()
    cp_wk.start()
    x_copy(0).start()
    cp_wv.start()
    x_copy(1).start()

    cp_wphi.wait()
    sr = lax.broadcasted_iota(jnp.int32, (32, 512), 0)
    sc = lax.broadcasted_iota(jnp.int32, (32, 512), 1)
    sel = jnp.where(sr == (sc // 16), 1.0, 0.0).astype(jnp.bfloat16)
    br = lax.broadcasted_iota(jnp.int32, (256, 512), 0)
    bc = lax.broadcasted_iota(jnp.int32, (256, 512), 1)
    bmat = jnp.where((br // 16) == (bc % 16), _dot(wphi_v[...], sel, _NN), 0.0).astype(jnp.bfloat16)
    er = lax.broadcasted_iota(jnp.int32, (128, 256), 0)
    ec = lax.broadcasted_iota(jnp.int32, (128, 256), 1)
    emat = jnp.where((er // 8) == (ec % 16), 1.0, 0.0).astype(jnp.bfloat16)
    tr = lax.broadcasted_iota(jnp.int32, (128, 512), 0)
    tc = lax.broadcasted_iota(jnp.int32, (128, 512), 1)
    tall = jnp.where((tr % 8) == ((tc // 16) % 8), _dot(emat, bmat, _NN), 0.0).astype(jnp.bfloat16)

    def fold(w_v, wT):
        for g in range(G):
            tg = tall[:, g * 128:(g + 1) * 128]
            w = _dot(tg, w_v[:, pl.ds(g * 128, 128)], _NT)
            w = w - jnp.mean(w, axis=-1, keepdims=True)
            wT[pl.ds(g * 128, 128), :] = w.astype(jnp.bfloat16)

    cp_wk.wait()
    fold(wk_v, wkT)

    def k_raw(t):
        xb = x_v[pl.ds(t * TS, TS), :]
        kT = _dot(wkT[...], xb, _NT)
        xf = xb.astype(jnp.float32)
        mu = jnp.mean(xf, axis=-1, keepdims=True)
        xc = xf - mu
        var = jnp.mean(xc * xc, axis=-1, keepdims=True)
        rc = lax.rsqrt(var + EPS)
        rr = jnp.broadcast_to(rc * LOG2E, (TS, 128)).T[0:8]
        r_v[t] = rr
        return kT, mu, rc, rr

    T2 = TS // 2

    def st_k(i):
        xb = x_v[pl.ds(i * T2, T2), :]
        kT = _dot(wkT[...], xb, _NT)
        xf = xb.astype(jnp.float32)
        mu = jnp.mean(xf, axis=-1, keepdims=True)
        xc = xf - mu
        var = jnp.mean(xc * xc, axis=-1, keepdims=True)
        rc = lax.rsqrt(var + EPS)
        rr = jnp.broadcast_to(rc * LOG2E, (T2, 128)).T[0:8]
        r_v[i // 2, :, pl.ds((i % 2) * T2, T2)] = rr
        return kT, mu, rc, rr

    def st_v(row0, n, mu, rc, wvs):
        vr = _dot(x_v[pl.ds(row0, n), :], wv_v[...], _NN)
        return ((vr - mu * wvs) * rc).astype(jnp.bfloat16)

    def st_kv(kT, rr, v, kvs, zs):
        n = kT.shape[-1]
        kvs_new, zs_new = [], []
        for g in range(G):
            pk = _feat(kT[g * 128:(g + 1) * 128], rr)
            zp = pk[:, 0:128]
            for j in range(1, n // 128):
                zp = zp + pk[:, j * 128:(j + 1) * 128]
            kv = _dot(pk.astype(jnp.bfloat16), v[:, g * 128:(g + 1) * 128], _NN)
            kvs_new.append(kv if kvs is None else kvs[g] + kv)
            zs_new.append(zp if zs is None else zs[g] + zp)
        return kvs_new, zs_new

    x_copy(0).wait()
    k0 = k_raw(0)
    cp_wv.wait()
    x_copy(1).wait()
    x_copy(2).start()
    x_copy(3).start()
    cp_wq.start()
    wvs = _dot(jnp.ones((8, D), jnp.bfloat16), wv_v[...], _NN)[0:1]
    ks = {0: k0}
    vs = {}
    kvs = zs = None
    vs[0] = st_v(0, TS, ks[0][1], ks[0][2], wvs)
    ks[2] = st_k(2)
    kvs, zs = st_kv(ks[0][0], ks[0][3], vs[0], kvs, zs)
    vs[2] = st_v(2 * T2, T2, ks[2][1], ks[2][2], wvs)
    ks[3] = st_k(3)
    kvs, zs = st_kv(ks[2][0], ks[2][3], vs[2], kvs, zs)
    vs[3] = st_v(3 * T2, T2, ks[3][1], ks[3][2], wvs)
    kvs, zs = st_kv(ks[3][0], ks[3][3], vs[3], kvs, zs)
    x_copy(2).wait()
    x_copy(3).wait()
    cp_wq.wait()
    cp_wo.start()
    cp_w1.start()
    cp_b1.start()
    cp_w2.start()
    cp_b2.start()
    ks[4] = st_k(4)
    ks[5] = st_k(5)
    ks[6] = st_k(6)
    ks[7] = st_k(7)
    vs[4] = st_v(4 * T2, T2, ks[4][1], ks[4][2], wvs)
    vs[5] = st_v(5 * T2, T2, ks[5][1], ks[5][2], wvs)
    vs[6] = st_v(6 * T2, T2, ks[6][1], ks[6][2], wvs)
    vs[7] = st_v(7 * T2, T2, ks[7][1], ks[7][2], wvs)
    fold(wq_v, wqT)
    kvs, zs = st_kv(ks[4][0], ks[4][3], vs[4], kvs, zs)
    kvs, zs = st_kv(ks[5][0], ks[5][3], vs[5], kvs, zs)
    kvs, zs = st_kv(ks[6][0], ks[6][3], vs[6], kvs, zs)
    kvs, zs = st_kv(ks[7][0], ks[7][3], vs[7], kvs, zs)
    for g in range(G):
        kv_s[g] = kvs[g]
        z_s[g] = zs[g]

    cp_wo.wait()
    cp_w1.wait()
    cp_b1.wait()
    cp_w2.wait()
    cp_b2.wait()

    def out_copy(i, c=None):
        s0 = i * TH if isinstance(i, int) else pl.multiple_of(i * TH, TH)
        if c is None:
            return pltpu.make_async_copy(out_v.at[pl.ds(s0, TH), :], out_hbm.at[pl.ds(s0, TH), :], osems.at[i])
        cs = pl.ds(c * (D // 2), D // 2)
        sem = osems.at[i] if c == 0 else osems.at[NT2 * NH + i // NH]
        return pltpu.make_async_copy(out_v.at[pl.ds(s0, TH), cs], out_hbm.at[pl.ds(s0, TH), cs], sem)

    def phase2(t, carry):
        rr_ = lax.broadcasted_iota(jnp.int32, (128, 256), 0)
        cc_ = lax.broadcasted_iota(jnp.int32, (128, 256), 1)
        m_kv = (rr_ // 16) == (cc_ % 8)
        lmats = [jnp.where(m_kv, kv_s[g].T, 0.0).astype(jnp.bfloat16) for g in range(G)]
        zbs = [jnp.broadcast_to(jnp.sum(z_s[g], axis=1, keepdims=True), (256, 128)) for g in range(G)]
        offs = [pl.multiple_of((t * NH + u) * TH, TH) for u in range(NH)]
        qTs = [_dot(wqT[...], x_v[pl.ds(s0, TH), :], _NT) for s0 in offs]
        oTs = []
        for u in range(NH):
            rr = r_v[t * (NH * TH // TS) + (u * TH) // TS, :, pl.ds((u * TH) % TS, TH)]
            parts = []
            for g in range(G):
                pq, den = _feat(qTs[u][g * 128:(g + 1) * 128], rr, zbs[g])
                nd = _dot(lmats[g], pq.astype(jnp.bfloat16), _NN)
                rden = 1.0 / (den + 1e-6)
                o3 = nd.reshape(8, 16, TH) * rden.reshape(8, 1, TH)
                parts.append(o3.reshape(128, TH).astype(jnp.bfloat16))
            oTs.append(jnp.concatenate(parts, axis=0))
        hs = []
        for u in range(NH):
            attn = _dot(oTs[u], wo_v[...], _TN)
            h = x_v[pl.ds(offs[u], TH), :].astype(jnp.float32) + attn
            hs.append((h, _ln(h).astype(jnp.bfloat16)))
        for u in range(NH):
            h, hn = hs[u]
            a = _dot(hn, w1_v[...], _NN) + b1_v[...].astype(jnp.float32).reshape(1, F)
            a = jnp.maximum(a, 0.0)
            a = (a * a).astype(jnp.bfloat16)
            if u < NH - 1:
                y = _dot(a, w2_v[...], _NN) + b2_v[...].astype(jnp.float32).reshape(1, D) + h
                out_v[pl.ds(offs[u], TH), :] = y.astype(jnp.bfloat16)
                out_copy(t * NH + u).start()
            else:
                b2f = b2_v[...].astype(jnp.float32).reshape(1, D)
                for c in range(2):
                    lo, hi = c * (D // 2), (c + 1) * (D // 2)
                    y = _dot(a, w2_v[:, pl.ds(lo, D // 2)], _NN) + b2f[:, lo:hi] + h[:, lo:hi]
                    out_v[pl.ds(offs[u], TH), pl.ds(lo, D // 2)] = y.astype(jnp.bfloat16)
                    out_copy(t * NH + u, c).start()
        return carry

    lax.fori_loop(0, NT2, phase2, 0)
    for i in range(NT2 * NH):
        if i % NH < NH - 1:
            out_copy(i).wait()
        else:
            out_copy(i, 0).wait()
            out_copy(i, 1).wait()


@jax.jit
def pallas_sequential_preLN__linear_kernel_hedgehog__dense_activation_squared_relu__prompt_kernel(
    A_x, A_wqkv, A_w_phi, A_wo, B_x, B_w1, B_b1, B_w2, B_b2,
):
    bf = jnp.bfloat16
    x2 = A_x.reshape(S, D)
    wphi2 = jnp.transpose(A_w_phi, (1, 2, 0)).reshape(DH * DH, H)
    any_spec = pl.BlockSpec(memory_space=pl.ANY)
    out = pl.pallas_call(
        _kernel,
        out_shape=jax.ShapeDtypeStruct((S, D), bf),
        in_specs=[any_spec] * 8,
        out_specs=any_spec,
        scratch_shapes=[
            pltpu.VMEM((S, D), bf),
            pltpu.VMEM((D, D), bf),
            pltpu.VMEM((D, D), bf),
            pltpu.VMEM((D, D), bf),
            pltpu.VMEM((DH * DH, H), bf),
            pltpu.VMEM((D, D), bf),
            pltpu.VMEM((D, F), bf),
            pltpu.VMEM((F,), bf),
            pltpu.VMEM((F, D), bf),
            pltpu.VMEM((D,), bf),
            pltpu.VMEM((D, D), bf),
            pltpu.VMEM((D, D), bf),
            pltpu.VMEM((NT, 8, TS), jnp.float32),
            pltpu.VMEM((G, 256, 128), jnp.float32),
            pltpu.VMEM((G, 256, 128), jnp.float32),
            pltpu.VMEM((S, D), bf),
            pltpu.SemaphoreType.DMA((9,)),
            pltpu.SemaphoreType.DMA((NT,)),
            pltpu.SemaphoreType.DMA((NT2 * NH + NT2,)),
        ],
        compiler_params=pltpu.CompilerParams(vmem_limit_bytes=100 * 1024 * 1024),
    )(x2, A_wqkv, wphi2, A_wo, B_w1, B_b1, B_w2, B_b2)
    return out.reshape(1, S, D)
```
